```python
import jax
import jax.numpy as jnp

def _softmax(x, axis=-1):
    return jax.nn.softmax(x, axis=axis)
def _gelu(x):
    return jax.nn.gelu(x, approximate=True)
def _silu(x):
    return jax.nn.silu(x)
def _sigmoid(x):
    return jax.nn.sigmoid(x)
def _layernorm(x, axis=-1, eps=1e-5):
    m = jnp.mean(x, axis=axis, keepdims=True)
    v = jnp.var(x, axis=axis, keepdims=True)
    return (x - m) / jnp.sqrt(v + eps)
def _scatter_add(tgt, idx, src, axis=0):
    return tgt.at[idx].add(src)
def _segment_sum(src, seg, n):
    return jax.ops.segment_sum(src, seg, n)
class _Rng:
    def __init__(self, key):
        self._k = key
    def _next(self):
        self._k, sub = jax.random.split(self._k)
        return sub
    def normal(self, shape):
        return jax.random.normal(self._next(), shape, dtype=jnp.bfloat16)
    def randint(self, lo, hi, shape):
        return jax.random.randint(self._next(), shape, lo, hi, dtype=jnp.int32)
    def uniform(self, shape, lo=0.0, hi=1.0):
        return jax.random.uniform(self._next(), shape, jnp.bfloat16, lo, hi)
    def permutation(self, n):
        return jax.random.permutation(self._next(), n)


kernel_name = 'parallel_sum__linear_kernel_hedgehog__glu_gated_bilinear__prompt'

def _fwd_setup_inputs():
    _rng = _Rng(jax.random.key(int.from_bytes(__import__("os").urandom(4), "little")))
    _w = (lambda a: (lambda t: t.astype(jnp.bfloat16) if jnp.issubdtype(t.dtype, jnp.floating) else t)(jnp.asarray(a)))
    def _A_setup():
        B, S, D, H = 1, 2048, 512, 32
        Dh = D // H
        return {
            "x": _w((lambda *s: _rng.normal(s) * 0.05)(B, S, D)),
            "wqkv": _w((lambda *s: _rng.normal(s) * 0.05)(D, 3 * D)),
            "w_phi": _w((lambda *s: _rng.normal(s) * 0.05)(H, Dh, Dh) * (Dh ** -0.5)),
            "wo": _w((lambda *s: _rng.normal(s) * 0.05)(D, D)),
        }
    _A_in = _A_setup()

    def _B_setup():
        B, S, D, F = 1, 2048, 512, 1792
        return {
            "x": _w((lambda *s: _rng.normal(s) * 0.05)(B, S, D)),
            "w_gate": _w((lambda *s: _rng.normal(s) * 0.05)(D, F) * (D ** -0.5)),
            "w_up": _w((lambda *s: _rng.normal(s) * 0.05)(D, F) * (D ** -0.5)),
            "w_down": _w((lambda *s: _rng.normal(s) * 0.05)(F, D) * (F ** -0.5)),
        }
    _B_in = _B_setup()

    return {
        "A_x": _A_in["x"],
        "A_wqkv": _A_in["wqkv"],
        "A_w_phi": _A_in["w_phi"],
        "A_wo": _A_in["wo"],
        "B_x": _B_in["x"],
        "B_w_gate": _B_in["w_gate"],
        "B_w_up": _B_in["w_up"],
        "B_w_down": _B_in["w_down"],
    }

def _fwd_reference(A_x, A_wqkv, A_w_phi, A_wo, B_x, B_w_gate, B_w_up, B_w_down):
    def _A_ref(x, wqkv, w_phi, wo):
        B, S, D = x.shape
        H = 32; Dh = D // H
        qkv = (lambda x, *d: x.transpose(*d))((x @ wqkv).reshape(B, S, 3, H, Dh), 2, 0, 3, 1, 4)
        q, k, v = qkv[0], qkv[1], qkv[2]
        pq = jnp.einsum("bhsd,hdf->bhsf", q, w_phi)
        pk = jnp.einsum("bhsd,hdf->bhsf", k, w_phi)
        phi_q = jnp.concatenate([_softmax(pq, axis=-1), _softmax(-pq, axis=-1)], axis=-1)
        phi_k = jnp.concatenate([_softmax(pk, axis=-1), _softmax(-pk, axis=-1)], axis=-1)
        kv = jnp.einsum("bhsf,bhsd->bhfd", phi_k, v)
        z  = jnp.einsum("bhsf->bhf", phi_k)
        num = jnp.einsum("bhqf,bhfd->bhqd", phi_q, kv)
        den = jnp.einsum("bhqf,bhf->bhq", phi_q, z)[..., None] + 1e-6
        o = num / den
        return (lambda x, *d: x.transpose(*d))(o, 0, 2, 1, 3).reshape(B, S, D) @ wo

    def _B_ref(x, w_gate, w_up, w_down):
        g = jnp.einsum("bsd,df->bsf", x, w_gate)
        u = jnp.einsum("bsd,df->bsf", x, w_up)
        h = g * u
        return jnp.einsum("bsf,fd->bsd", h, w_down)

    x = A_x
    xn = _layernorm(x, axis=-1)
    return x + _A_ref(xn, A_wqkv, A_w_phi, A_wo) + _B_ref(xn, B_w_gate, B_w_up, B_w_down)


def setup_inputs():
    _inp = _fwd_setup_inputs()
    _gk = jax.random.fold_in(jax.random.key(int.from_bytes(__import__("os").urandom(4), "little")), 2**31 - 1)
    _shapes = [[1, 2048, 512]]
    _dtypes = ['bfloat16']
    _gks = jax.random.split(_gk, len(_shapes))
    _gs = [jax.random.normal(k, s, dtype=jnp.dtype(d)) * 0.05 for k, s, d in zip(_gks, _shapes, _dtypes)]
    _inp["grad_out"] = _gs[0]
    return _inp

def reference(A_x, A_wqkv, A_w_phi, A_wo, B_w_gate, B_w_up, B_w_down, B_x, grad_out):
    _const = dict(B_x=B_x)
    def _f(*_d):
        return _fwd_reference(**{'A_x': _d[0], 'A_wqkv': _d[1], 'A_w_phi': _d[2], 'A_wo': _d[3], 'B_w_gate': _d[4], 'B_w_up': _d[5], 'B_w_down': _d[6], **_const})
    _out, _vjp = jax.vjp(_f, A_x, A_wqkv, A_w_phi, A_wo, B_w_gate, B_w_up, B_w_down)
    _grads = _vjp(grad_out)
    _out0 = jnp.asarray(_out)
    return (_out0, *[jnp.asarray(_g) for _g in _grads])
```

```python
import jax
import jax.numpy as jnp
from jax import lax
import jax.experimental.pallas as pl
import jax.experimental.pallas.tpu as pltpu

S = 2048
D = 512
H = 32
DH = 16
F = 1792
G = 4
U = 8
E = 80
T = 256
NT_ = S // T
WC = 256
NWC = F // WC
FC = 256
F32 = jnp.float32
BF16 = jnp.bfloat16
LOG2E = 1.4426950408889634


def _nn(a, b):
    return jnp.dot(a, b, preferred_element_type=F32)


def _nt(a, b):
    return lax.dot_general(a, b, (((1,), (1,)), ((), ())), preferred_element_type=F32)


def _tn(a, b):
    return lax.dot_general(a, b, (((0,), (0,)), ((), ())), preferred_element_type=F32)


def _loop(n, fn):
    def body(i, c):
        fn(i)
        return c
    lax.fori_loop(0, n, body, 0)


def _iota2(shape):
    return lax.broadcasted_iota(jnp.int32, shape, 0), lax.broadcasted_iota(jnp.int32, shape, 1)


def _onehot(cond):
    return jnp.where(cond, 1.0, 0.0).astype(BF16)


def _perm_head(p):
    return (p // 64) * 4 + p % 4


def _perm_feat(p):
    return ((p % 64) // 8) * 2 + (p % 8) // 4


def _fold(x):
    return pltpu.roll(x, 4, x.ndim - 2)


def _kernel(x_hbm, wqkv_hbm, wphi_hbm, wo_hbm, wg_hbm, wu_hbm, wd_hbm, dy_hbm,
            out_hbm, dx_hbm, dwqkv_hbm, dwphi_hbm, dwo_hbm, dwg_hbm, dwu_hbm, dwd_hbm,
            x_v, dy_v, wqkv_v, wphi_v, wo_v, wg_v, wu_v, wd_v,
            xn_v, xnT_v, rstd_v, weffT_v, weffS_v, wop_v, bT_v,
            phik_v, vT_v, phiq_v, oT_v, dT_v, dnum_v, pq_v,
            kv_acc, kv_b, kvT_b, dkv_acc, dkv_b, dkvT_b,
            h_v, dg_v, du_v,
            tmp_a, doT_v, tmp_c, c_acc, dxn_v,
            out_v, dx_v, dwqkv_v, dwphi_v, dwo_v, dwg_v, dwu_v, dwd_v,
            sems):
    def rows(src, dst, r0, n, s):
        return pltpu.make_async_copy(src.at[pl.ds(r0, n)], dst.at[pl.ds(r0, n)], sems.at[s])

    def cols(src, dst, c0, n, s):
        return pltpu.make_async_copy(src.at[:, pl.ds(c0, n)], dst.at[:, pl.ds(c0, n)], sems.at[s])

    def full(src, dst, s):
        return pltpu.make_async_copy(src, dst, sems.at[s])

    c_wphi = full(wphi_hbm, wphi_v, 0)
    c_x0 = rows(x_hbm, x_v, 0, T, 1)
    c_wk = cols(wqkv_hbm, wqkv_v, D, D, 2)
    c_wv = cols(wqkv_hbm, wqkv_v, 2 * D, D, 3)
    c_x1 = rows(x_hbm, x_v, T, T, 4)
    c_wq = cols(wqkv_hbm, wqkv_v, 0, D, 4)

    def c_xt(t):
        return pltpu.make_async_copy(x_hbm.at[pl.ds(t * T, T)], x_v.at[pl.ds(t * T, T)], sems.at[5 + t])
    c_late = [full(wo_hbm, wo_v, 5), full(dy_hbm, dy_v, 5), full(wg_hbm, wg_v, 5),
              full(wu_hbm, wu_v, 5), full(wd_hbm, wd_v, 5)]
    out_copies = []

    def emit(c):
        c.start()
        out_copies.append(c)

    c_wphi.start()
    c_x0.start()
    c_wk.start()
    c_wv.start()
    c_x1.start()
    c_wq.start()

    r128, c128 = _iota2((128, 128))
    pt_mat = _onehot(_perm_head(r128) * 16 + _perm_feat(r128) == c128)
    p_mat = _onehot(_perm_head(c128) * 16 + _perm_feat(c128) == r128)

    kv_acc[...] = jnp.zeros_like(kv_acc)
    dkv_acc[...] = jnp.zeros_like(dkv_acc)
    rx = lax.broadcasted_iota(jnp.int32, (16, S), 0)
    ones_rows = _onehot(rx < 8)
    for u in range(U):
        vT_v[u * E + 64:(u + 1) * E, :] = ones_rows
        dnum_v[u * E + 64:(u + 1) * E, :] = jnp.zeros((16, T), BF16)

    c_wphi.wait()
    c_x0.wait()
    w2 = wphi_v[...].reshape(DH * DH, H)
    rs, cs_ = _iota2((H, D))
    sel = _onehot(rs == cs_ // 16)
    ry, cy = _iota2((DH * DH, D))
    y = jnp.where(ry // 16 == cy % 16, _nn(w2, sel), 0.0).astype(BF16)
    rr, cr = _iota2((128, DH * DH))
    rsel = _onehot(_perm_feat(rr) == cr % 16)
    rb, cb = _iota2((128, D))
    ball = jnp.where(_perm_head(rb) == (cb // 16) % 8, _nn(rsel, y), 0.0).astype(BF16)
    for g in range(G):
        bT_v[g] = ball[:, g * 128:(g + 1) * 128]
        bT_v[G + g] = ball[:, g * 128:(g + 1) * 128]
        bT_v[2 * G + g] = pt_mat

    def ln_tile(t):
        r0 = pl.multiple_of(t * T, T)
        xx = x_v[pl.ds(r0, T), :].astype(F32)
        m = jnp.mean(xx, axis=-1, keepdims=True)
        xc = xx - m
        var = jnp.mean(xc * xc, axis=-1, keepdims=True)
        rstd = lax.rsqrt(var + 1e-5)
        xn = xc * rstd
        rstd_v[pl.ds(r0, T), :] = rstd
        xn_v[pl.ds(r0, T), :] = xn.astype(BF16)
        xnT_v[:, pl.ds(r0, T)] = xn.T.astype(BF16)

    ln_tile(0)

    def prep(p):
        for b in range(4 * p, 4 * p + 4):
            w = _nt(bT_v[b], wqkv_v[:, b * 128:(b + 1) * 128])
            weffT_v[b * 128:(b + 1) * 128, :] = w.astype(BF16)
            if b < 8:
                weffS_v[b * 128:(b + 1) * 128, :] = (w * LOG2E).astype(BF16)


    def softmax_store(src_ref, src_c0, dst_ref, dst_c0, us=range(U)):
        for u in us:
            a = src_ref[u * 64:(u + 1) * 64, pl.ds(src_c0, T)].reshape(8, 8, T)
            mx = jnp.max(a, axis=0)
            mx = jnp.maximum(mx, _fold(mx))
            mn = jnp.min(a, axis=0)
            mn = jnp.minimum(mn, _fold(mn))
            ep = jnp.exp2(a - mx[None])
            en = jnp.exp2(mn[None] - a)
            sp = jnp.sum(ep, axis=0)
            sn = jnp.sum(en, axis=0)
            rp = 1.0 / (sp + _fold(sp))
            rn = 1.0 / (sn + _fold(sn))
            cs = pl.ds(dst_c0, T)
            dst_ref[u * 128: u * 128 + 64, cs] = (ep * rp[None]).reshape(64, T).astype(BF16)
            dst_ref[u * 128 + 64: u * 128 + 128, cs] = (en * rn[None]).reshape(64, T).astype(BF16)

    def pq_mm(t):
        c0 = pl.multiple_of(t * T, T)
        pq_v[:, pl.ds(c0, T)] = _nn(weffS_v[0:512, :], xnT_v[:, pl.ds(c0, T)])

    def pk_mm(t):
        c0 = pl.multiple_of(t * T, T)
        tmp_a[0:512, :] = _nn(weffS_v[512:1024, :], xnT_v[:, pl.ds(c0, T)])

    def v_mm(t):
        c0 = pl.multiple_of(t * T, T)
        vv = _nn(weffT_v[1024:1536, :], xnT_v[:, pl.ds(c0, T)]).astype(BF16)
        for u in range(U):
            vT_v[u * E: u * E + 64, pl.ds(c0, T)] = vv[u * 64:(u + 1) * 64, :]

    def kv_mm(t):
        c0 = pl.multiple_of(t * T, T)
        for u in range(U):
            kv_acc[u, 0:E, :] += _nt(vT_v[u * E:(u + 1) * E, pl.ds(c0, T)], phik_v[u * 128:(u + 1) * 128, pl.ds(c0, T)])

    c_wk.wait()
    for t in range(2, NT_):
        c_xt(t).start()
    prep(1)
    pk_mm(0)
    c_wv.wait()
    prep(2)
    softmax_store(tmp_a, 0, phik_v, 0)
    v_mm(0)
    c_x1.wait()
    c_wq.wait()
    prep(0)
    kv_mm(0)
    ln_tile(1)
    for c in c_late:
        c.start()

    def phase_a(i):
        t = i + 1

        @pl.when(t + 1 < NT_)
        def _():
            c_xt(t + 1).wait()
        pk_mm(t)
        v_mm(t)
        pq_mm(t - 1)
        ln_tile(jnp.minimum(t + 1, NT_ - 1))
        softmax_store(tmp_a, 0, phik_v, pl.multiple_of(t * T, T))
        kv_mm(t)

    _loop(NT_ - 1, phase_a)

    mask_kvT = (r128 % 4 == c128 % 4) & (r128 < 72)
    mask_kv = (r128 % 4 == c128 % 4) & (c128 < 68)

    def finish_kv(acc, b_ref, bT_ref):
        for u in range(U):
            a = acc[u]
            bT_ref[u] = jnp.where(mask_kvT, a, 0.0)[0:E, :].astype(BF16)
            at = a.T.reshape(2, 8, 8, 128)
            s1 = jnp.sum(at, axis=1)
            mean = (s1 + _fold(s1)) * (1.0 / 16.0)
            atc = (at - mean[:, None]).reshape(128, 128)
            b_ref[u] = jnp.where(mask_kv, atc, 0.0).astype(BF16)

    for c in c_late:
        c.wait()
    for g in range(G):
        wop_v[g * 128:(g + 1) * 128, :] = _nn(pt_mat, wo_v[g * 128:(g + 1) * 128, :]).astype(BF16)
    pq_mm(NT_ - 1)
    finish_kv(kv_acc, kv_b, kvT_b)
    for t in range(4):
        doT_v[:, t * 512:(t + 1) * 512] = _nt(wop_v[...], dy_v[t * 512:(t + 1) * 512, :])

    def softmax_bwd(dphi_ref, phi_ref, phi_c0, u):
        cs = pl.ds(phi_c0, T)
        pp = phi_ref[u * 128: u * 128 + 64, cs].astype(F32).reshape(8, 8, T)
        pn = phi_ref[u * 128 + 64: u * 128 + 128, cs].astype(F32).reshape(8, 8, T)
        dpp = dphi_ref[u * 128: u * 128 + 64, :].reshape(8, 8, T)
        dpn = dphi_ref[u * 128 + 64: u * 128 + 128, :].reshape(8, 8, T)
        sp = jnp.sum(dpp * pp, axis=0)
        sn = jnp.sum(dpn * pn, axis=0)
        sp = sp + _fold(sp)
        sn = sn + _fold(sn)
        da = pp * (dpp - sp[None]) - pn * (dpn - sn[None])
        return da.reshape(64, T).astype(BF16)

    def ffn_units(r0):
        st = {}

        def ug(k):
            st[k, 'g'] = _nn(xn_v[pl.ds(r0, T), :], wg_v[:, k * FC:(k + 1) * FC])

        def uu(k):
            st[k, 'u'] = _nn(xn_v[pl.ds(r0, T), :], wu_v[:, k * FC:(k + 1) * FC])

        def ud(k):
            dh = _nt(dy_v[pl.ds(r0, T), :], wd_v[k * FC:(k + 1) * FC, :])
            gg, uv = st[k, 'g'], st[k, 'u']
            h_v[pl.ds(r0, T), k * FC:(k + 1) * FC] = (gg * uv).astype(BF16)
            dg_v[pl.ds(r0, T), k * FC:(k + 1) * FC] = (dh * uv).astype(BF16)
            du_v[pl.ds(r0, T), k * FC:(k + 1) * FC] = (dh * gg).astype(BF16)

        units = []
        for k in range(F // FC):
            units += [lambda k=k: ug(k), lambda k=k: uu(k), lambda k=k: ud(k)]
        return units

    def phase_b(t):
        c0 = pl.multiple_of(t * T, T)
        units = ffn_units(c0)

        def s1(u):
            softmax_store(pq_v, c0, phiq_v, 0, (u,))
            tmp_c[u] = _nn(kvT_b[u], phiq_v[u * 128:(u + 1) * 128, :])

        def s2(u):
            num = tmp_c[u, 0:64, :].reshape(8, 8, T)
            rden = 1.0 / (tmp_c[u, 64:72, :] + 1e-6)
            o = num * rden[None]
            dnum = doT_v[u * 64:(u + 1) * 64, pl.ds(c0, T)].reshape(8, 8, T) * rden[None]
            dd = jnp.sum(dnum * o, axis=0)
            dden = -(dd + _fold(dd))
            oT_v[u * 64:(u + 1) * 64, pl.ds(c0, T)] = o.reshape(64, T).astype(BF16)
            dnum_v[u * E: u * E + 64, :] = dnum.reshape(64, T).astype(BF16)
            dnum_v[u * E + 64: u * E + 72, :] = dden.astype(BF16)
            dn = dnum_v[u * E:(u + 1) * E, :]
            tmp_a[u * 128:(u + 1) * 128, :] = _nn(kv_b[u, :, 0:E], dn)
            dkv_acc[u, 0:E, :] += _nt(dn, phiq_v[u * 128:(u + 1) * 128, :])

        def s3(u):
            dT_v[u * 64:(u + 1) * 64, pl.ds(c0, T)] = softmax_bwd(tmp_a, phiq_v, 0, u)

        for i, un in enumerate(units):
            un()
            if i % 2 == 0 and i // 2 < U:
                s1(i // 2)
            if i % 2 == 1 and 1 <= i // 2 < U + 1:
                s2(i // 2 - 1)
            if i % 2 == 0 and 2 <= i // 2 < U + 2:
                s3(i // 2 - 2)

    _loop(NT_, phase_b)

    def meff(part):
        return _nt(xnT_v[...], dT_v[part * 512:(part + 1) * 512, :]).astype(BF16)

    def small(part, me):
        for g in range(G):
            mb = me[:, g * 128:(g + 1) * 128]
            sl = slice(part * 512 + g * 128, part * 512 + (g + 1) * 128)
            dwqkv_v[:, sl] = _nn(mb, bT_v[part * G + g]).astype(BF16)
            if part < 2:
                c_acc[part, g * 128:(g + 1) * 128, :] = _tn(wqkv_v[:, sl], mb)

    mq = meff(0)
    finish_kv(dkv_acc, dkv_b, dkvT_b)
    dxn_v[1] = jnp.zeros((T, D), F32)
    dwop = _nn(oT_v[...], dy_v[...]).astype(BF16)
    small(0, mq)
    for g in range(G):
        dwo_v[g * 128:(g + 1) * 128, :] = _nn(p_mat, dwop[g * 128:(g + 1) * 128, :]).astype(BF16)
    emit(full(dwo_v, dwo_hbm, 0))

    def dx_epi(t):
        r0 = pl.multiple_of(t * T, T)
        dxn = dxn_v[t % 2]
        xn = xn_v[pl.ds(r0, T), :].astype(F32)
        m1 = jnp.mean(dxn, axis=-1, keepdims=True)
        m2 = jnp.mean(dxn * xn, axis=-1, keepdims=True)
        dx = dy_v[pl.ds(r0, T), :].astype(F32) + rstd_v[pl.ds(r0, T), :] * (dxn - m1 - xn * m2)
        dx_v[pl.ds(r0, T), :] = dx.astype(BF16)

    def phase_c(t):
        c0 = pl.multiple_of(t * T, T)
        for u in range(U):
            tmp_a[u * 128:(u + 1) * 128, :] = _nn(dkv_b[u, :, 0:E], vT_v[u * E:(u + 1) * E, pl.ds(c0, T)])
            dT_v[1024 + u * 64: 1024 + (u + 1) * 64, pl.ds(c0, T)] = _nn(
                dkvT_b[u, 0:64, :], phik_v[u * 128:(u + 1) * 128, pl.ds(c0, T)]).astype(BF16)
        for u in range(U):
            dT_v[512 + u * 64: 512 + (u + 1) * 64, pl.ds(c0, T)] = softmax_bwd(tmp_a, phik_v, c0, u)
        y = _nn(h_v[pl.ds(c0, T), :], wd_v[...]) + _tn(oT_v[:, pl.ds(c0, T)], wop_v[...])
        out_v[pl.ds(c0, T), :] = (x_v[pl.ds(c0, T), :].astype(F32) + y).astype(BF16)
        dx_epi(jnp.maximum(t - 1, 0) + (t == 0).astype(jnp.int32))
        dxn_v[t % 2] = (_tn(dT_v[:, pl.ds(c0, T)], weffT_v[...])
                        + _nt(dg_v[pl.ds(c0, T), :], wg_v[...]) + _nt(du_v[pl.ds(c0, T), :], wu_v[...]))

    _loop(NT_, phase_c)
    emit(full(out_v, out_hbm, 0))
    emit(rows(dx_v, dx_hbm, 0, S - T, 0))

    def wg_mm(f0, n=WC):
        dwg_v[:, pl.ds(f0, n)] = _nn(xnT_v[...], dg_v[:, pl.ds(f0, n)]).astype(BF16)

    def wu_mm(f0, n=WC):
        dwu_v[:, pl.ds(f0, n)] = _nn(xnT_v[...], du_v[:, pl.ds(f0, n)]).astype(BF16)

    def wd_mm(f0, n=WC):
        dwd_v[pl.ds(f0, n), :] = _tn(h_v[:, pl.ds(f0, n)], dy_v[...]).astype(BF16)

    dx_epi(NT_ - 1)
    mk = meff(1)
    mv = meff(2)
    small(1, mk)
    wg_mm(0)
    small(2, mv)
    rc, cc = _iota2((D, 128))
    cm = jnp.where((rc // 16) % 8 == _perm_head(cc), c_acc[0] + c_acc[1], 0.0).astype(BF16)
    re_, ce = _iota2((128, DH * DH))
    e3 = _onehot(_perm_feat(re_) == ce % 16)
    ra, ca = _iota2((D, DH * DH))
    a2 = jnp.where(ra % 16 == ca // 16, _nn(cm, e3), 0.0).astype(BF16)
    wu_mm(0)
    rh, ch = _iota2((D, H))
    r2t = _onehot(rh // 16 == ch)
    dwphi_v[...] = _tn(a2, r2t).astype(BF16).reshape(DH, DH, H)
    wd_mm(0)
    emit(rows(dx_v, dx_hbm, S - T, T, 0))
    emit(full(dwqkv_v, dwqkv_hbm, 0))
    emit(full(dwphi_v, dwphi_hbm, 0))

    def wgrad(i):
        f0 = pl.multiple_of((i + 1) * WC, WC)
        wg_mm(f0)
        wu_mm(f0)
        wd_mm(f0)

    _loop(NWC - 2, wgrad)

    fl = (NWC - 1) * WC
    emit(cols(dwg_v, dwg_hbm, 0, fl, 0))
    emit(cols(dwu_v, dwu_hbm, 0, fl, 0))
    emit(rows(dwd_v, dwd_hbm, 0, fl, 0))
    wg_mm(fl)
    emit(cols(dwg_v, dwg_hbm, fl, WC, 0))
    wd_mm(fl)
    emit(rows(dwd_v, dwd_hbm, fl, WC, 0))
    for k in range(2):
        wu_mm(fl + k * 128, 128)
        emit(cols(dwu_v, dwu_hbm, fl + k * 128, 128, 0))

    for c in out_copies:
        c.wait()


@jax.jit
def pallas_parallel_sum__linear_kernel_hedgehog__glu_gated_bilinear__prompt_kernel(
    A_x: jax.Array,
    A_wqkv: jax.Array,
    A_w_phi: jax.Array,
    A_wo: jax.Array,
    B_x: jax.Array,
    B_w_gate: jax.Array,
    B_w_up: jax.Array,
    B_w_down: jax.Array,
    grad_out: jax.Array,
):
    del B_x
    x2 = A_x.reshape(S, D)
    dy2 = grad_out.reshape(S, D)
    wphi_t = jnp.transpose(A_w_phi, (1, 2, 0))

    vm = pltpu.VMEM
    scratch = [
        vm((S, D), BF16), vm((S, D), BF16), vm((D, 3 * D), BF16), vm((DH, DH, H), BF16), vm((D, D), BF16),
        vm((D, F), BF16), vm((D, F), BF16), vm((F, D), BF16),
        vm((S, D), BF16), vm((D, S), BF16), vm((S, 1), F32), vm((3 * D, D), BF16), vm((2 * D, D), BF16),
        vm((D, D), BF16), vm((3 * G, 128, 128), BF16),
        vm((1024, S), BF16), vm((U * E, S), BF16), vm((1024, T), BF16), vm((D, S), BF16), vm((3 * D, S), BF16),
        vm((U * E, T), BF16), vm((D, S), F32),
        vm((U, 128, 128), F32), vm((U, 128, 128), BF16), vm((U, E, 128), BF16),
        vm((U, 128, 128), F32), vm((U, 128, 128), BF16), vm((U, E, 128), BF16),
        vm((S, F), BF16), vm((S, F), BF16), vm((S, F), BF16),
        vm((1024, T), F32), vm((D, S), F32), vm((U, E, T), F32), vm((2, D, 128), F32),
        vm((2, T, D), F32),
        vm((S, D), BF16), vm((S, D), BF16), vm((D, 3 * D), BF16), vm((DH, DH, H), BF16), vm((D, D), BF16),
        vm((D, F), BF16), vm((D, F), BF16), vm((F, D), BF16),
        pltpu.SemaphoreType.DMA((5 + NT_,)),
    ]
    out_shape = (
        jax.ShapeDtypeStruct((S, D), BF16), jax.ShapeDtypeStruct((S, D), BF16),
        jax.ShapeDtypeStruct((D, 3 * D), BF16), jax.ShapeDtypeStruct((DH, DH, H), BF16),
        jax.ShapeDtypeStruct((D, D), BF16), jax.ShapeDtypeStruct((D, F), BF16),
        jax.ShapeDtypeStruct((D, F), BF16), jax.ShapeDtypeStruct((F, D), BF16),
    )
    anyspec = pl.BlockSpec(memory_space=pl.ANY)
    res = pl.pallas_call(
        _kernel,
        in_specs=[anyspec] * 8,
        out_specs=tuple([anyspec] * 8),
        out_shape=out_shape,
        scratch_shapes=scratch,
        compiler_params=pltpu.CompilerParams(vmem_limit_bytes=120 * 1024 * 1024),
    )(x2, A_wqkv, wphi_t, A_wo, B_w_gate, B_w_up, B_w_down, dy2)
    out, dx = res[0].reshape(1, S, D), res[1].reshape(1, S, D)
    dwphi = jnp.transpose(res[3], (2, 0, 1))
    return (out, dx, res[2], dwphi) + tuple(res[4:])
```

```python
import jax
import jax.numpy as jnp
from jax import lax
import jax.experimental.pallas as pl
import jax.experimental.pallas.tpu as pltpu

S = 2048
D = 512
H = 32
DH = 16
F = 1792
G = 4
U = 8
E = 80
T = 256
NT_ = S // T
WC = 256
NWC = F // WC
FC = 256
F32 = jnp.float32
BF16 = jnp.bfloat16
LOG2E = 1.4426950408889634


def _nn(a, b):
    return jnp.dot(a, b, preferred_element_type=F32)


def _nt(a, b):
    return lax.dot_general(a, b, (((1,), (1,)), ((), ())), preferred_element_type=F32)


def _tn(a, b):
    return lax.dot_general(a, b, (((0,), (0,)), ((), ())), preferred_element_type=F32)


def _loop(n, fn):
    def body(i, c):
        fn(i)
        return c
    lax.fori_loop(0, n, body, 0)


def _iota2(shape):
    return lax.broadcasted_iota(jnp.int32, shape, 0), lax.broadcasted_iota(jnp.int32, shape, 1)


def _onehot(cond):
    return jnp.where(cond, 1.0, 0.0).astype(BF16)


def _perm_head(p):
    return (p // 64) * 4 + p % 4


def _perm_feat(p):
    return ((p % 64) // 8) * 2 + (p % 8) // 4


def _fold(x):
    return pltpu.roll(x, 4, x.ndim - 2)


def _kernel(x_hbm, wqkv_hbm, wphi_hbm, wo_hbm, wg_hbm, wu_hbm, wd_hbm, dy_hbm,
            out_hbm, dx_hbm, dwqkv_hbm, dwphi_hbm, dwo_hbm, dwg_hbm, dwu_hbm, dwd_hbm,
            x_v, dy_v, wqkv_v, wphi_v, wo_v, wg_v, wu_v, wd_v,
            xn_v, xnT_v, rstd_v, weffT_v, weffS_v, wop_v, bT_v,
            phik_v, vT_v, phiq_v, oT_v, dT_v, dnum_v, pq_v,
            kv_acc, kv_b, kvT_b, dkv_acc, dkv_b, dkvT_b,
            h_v, dg_v, du_v,
            tmp_a, doT_v, tmp_c, c_acc, dxn_v,
            out_v, dx_v, dwqkv_v, dwphi_v, dwo_v, dwg_v, dwu_v, dwd_v,
            sems):
    def rows(src, dst, r0, n, s):
        return pltpu.make_async_copy(src.at[pl.ds(r0, n)], dst.at[pl.ds(r0, n)], sems.at[s])

    def cols(src, dst, c0, n, s):
        return pltpu.make_async_copy(src.at[:, pl.ds(c0, n)], dst.at[:, pl.ds(c0, n)], sems.at[s])

    def full(src, dst, s):
        return pltpu.make_async_copy(src, dst, sems.at[s])

    c_wphi = full(wphi_hbm, wphi_v, 0)
    c_x0 = rows(x_hbm, x_v, 0, T, 1)
    c_wk = cols(wqkv_hbm, wqkv_v, D, D, 2)
    c_wv = cols(wqkv_hbm, wqkv_v, 2 * D, D, 3)
    c_x1 = rows(x_hbm, x_v, T, T, 4)
    c_wq = cols(wqkv_hbm, wqkv_v, 0, D, 4)

    def c_xt(t):
        return pltpu.make_async_copy(x_hbm.at[pl.ds(t * T, T)], x_v.at[pl.ds(t * T, T)], sems.at[5 + t])
    c_late = [full(wo_hbm, wo_v, 5), full(dy_hbm, dy_v, 5), full(wg_hbm, wg_v, 5),
              full(wu_hbm, wu_v, 5), full(wd_hbm, wd_v, 5)]
    out_copies = []

    def emit(c):
        c.start()
        out_copies.append(c)

    c_wphi.start()
    c_x0.start()
    c_wk.start()
    c_wv.start()
    c_x1.start()
    c_wq.start()

    r128, c128 = _iota2((128, 128))
    pt_mat = _onehot(_perm_head(r128) * 16 + _perm_feat(r128) == c128)
    p_mat = _onehot(_perm_head(c128) * 16 + _perm_feat(c128) == r128)

    kv_acc[...] = jnp.zeros_like(kv_acc)
    dkv_acc[...] = jnp.zeros_like(dkv_acc)
    rx = lax.broadcasted_iota(jnp.int32, (16, S), 0)
    ones_rows = _onehot(rx < 8)
    for u in range(U):
        vT_v[u * E + 64:(u + 1) * E, :] = ones_rows
        dnum_v[u * E + 64:(u + 1) * E, :] = jnp.zeros((16, T), BF16)

    c_wphi.wait()
    c_x0.wait()
    w2 = wphi_v[...].reshape(DH * DH, H)
    rs, cs_ = _iota2((H, D))
    sel = _onehot(rs == cs_ // 16)
    ry, cy = _iota2((DH * DH, D))
    y = jnp.where(ry // 16 == cy % 16, _nn(w2, sel), 0.0).astype(BF16)
    rr, cr = _iota2((128, DH * DH))
    rsel = _onehot(_perm_feat(rr) == cr % 16)
    rb, cb = _iota2((128, D))
    ball = jnp.where(_perm_head(rb) == (cb // 16) % 8, _nn(rsel, y), 0.0).astype(BF16)
    for g in range(G):
        bT_v[g] = ball[:, g * 128:(g + 1) * 128]
        bT_v[G + g] = ball[:, g * 128:(g + 1) * 128]
        bT_v[2 * G + g] = pt_mat

    def ln_tile(t):
        r0 = pl.multiple_of(t * T, T)
        xx = x_v[pl.ds(r0, T), :].astype(F32)
        m = jnp.mean(xx, axis=-1, keepdims=True)
        xc = xx - m
        var = jnp.mean(xc * xc, axis=-1, keepdims=True)
        rstd = lax.rsqrt(var + 1e-5)
        xn = xc * rstd
        rstd_v[pl.ds(r0, T), :] = rstd
        xn_v[pl.ds(r0, T), :] = xn.astype(BF16)
        xnT_v[:, pl.ds(r0, T)] = xn.T.astype(BF16)

    ln_tile(0)

    def prep(p):
        for b in range(4 * p, 4 * p + 4):
            w = _nt(bT_v[b], wqkv_v[:, b * 128:(b + 1) * 128])
            weffT_v[b * 128:(b + 1) * 128, :] = w.astype(BF16)
            if b < 8:
                weffS_v[b * 128:(b + 1) * 128, :] = (w * LOG2E).astype(BF16)


    def softmax_store(src_ref, src_c0, dst_ref, dst_c0, us=range(U)):
        for u in us:
            a = src_ref[u * 64:(u + 1) * 64, pl.ds(src_c0, T)].reshape(8, 8, T)
            mx = jnp.max(a, axis=0)
            mx = jnp.maximum(mx, _fold(mx))
            mn = jnp.min(a, axis=0)
            mn = jnp.minimum(mn, _fold(mn))
            ep = jnp.exp2(a - mx[None])
            en = jnp.exp2(mn[None] - a)
            sp = jnp.sum(ep, axis=0)
            sn = jnp.sum(en, axis=0)
            rp = 1.0 / (sp + _fold(sp))
            rn = 1.0 / (sn + _fold(sn))
            cs = pl.ds(dst_c0, T)
            dst_ref[u * 128: u * 128 + 64, cs] = (ep * rp[None]).reshape(64, T).astype(BF16)
            dst_ref[u * 128 + 64: u * 128 + 128, cs] = (en * rn[None]).reshape(64, T).astype(BF16)

    def pq_mm(t):
        c0 = pl.multiple_of(t * T, T)
        pq_v[:, pl.ds(c0, T)] = _nn(weffS_v[0:512, :], xnT_v[:, pl.ds(c0, T)])

    def pk_mm(t):
        c0 = pl.multiple_of(t * T, T)
        tmp_a[0:512, :] = _nn(weffS_v[512:1024, :], xnT_v[:, pl.ds(c0, T)])

    def v_mm(t):
        c0 = pl.multiple_of(t * T, T)
        vv = _nn(weffT_v[1024:1536, :], xnT_v[:, pl.ds(c0, T)]).astype(BF16)
        for u in range(U):
            vT_v[u * E: u * E + 64, pl.ds(c0, T)] = vv[u * 64:(u + 1) * 64, :]

    def kv_mm(t):
        c0 = pl.multiple_of(t * T, T)
        for u in range(U):
            kv_acc[u, 0:E, :] += _nt(vT_v[u * E:(u + 1) * E, pl.ds(c0, T)], phik_v[u * 128:(u + 1) * 128, pl.ds(c0, T)])

    c_wk.wait()
    for t in range(2, NT_):
        c_xt(t).start()
    prep(1)
    pk_mm(0)
    c_wv.wait()
    prep(2)
    softmax_store(tmp_a, 0, phik_v, 0)
    v_mm(0)
    c_x1.wait()
    c_wq.wait()
    prep(0)
    kv_mm(0)
    ln_tile(1)
    for c in c_late:
        c.start()

    def phase_a(i):
        t = i + 1

        @pl.when(t + 1 < NT_)
        def _():
            c_xt(t + 1).wait()
        pk_mm(t)
        v_mm(t)
        pq_mm(t - 1)
        ln_tile(jnp.minimum(t + 1, NT_ - 1))
        softmax_store(tmp_a, 0, phik_v, pl.multiple_of(t * T, T))
        kv_mm(t)

    _loop(NT_ - 1, phase_a)

    mask_kvT = (r128 % 4 == c128 % 4) & (r128 < 72)
    mask_kv = (r128 % 4 == c128 % 4) & (c128 < 68)

    def finish_kv(acc, b_ref, bT_ref):
        for u in range(U):
            a = acc[u]
            bT_ref[u] = jnp.where(mask_kvT, a, 0.0)[0:E, :].astype(BF16)
            at = a.T.reshape(2, 8, 8, 128)
            s1 = jnp.sum(at, axis=1)
            mean = (s1 + _fold(s1)) * (1.0 / 16.0)
            atc = (at - mean[:, None]).reshape(128, 128)
            b_ref[u] = jnp.where(mask_kv, atc, 0.0).astype(BF16)

    for c in c_late:
        c.wait()
    for g in range(G):
        wop_v[g * 128:(g + 1) * 128, :] = _nn(pt_mat, wo_v[g * 128:(g + 1) * 128, :]).astype(BF16)
    pq_mm(NT_ - 1)
    finish_kv(kv_acc, kv_b, kvT_b)
    for t in range(4):
        doT_v[:, t * 512:(t + 1) * 512] = _nt(wop_v[...], dy_v[t * 512:(t + 1) * 512, :])

    def softmax_bwd(dphi_ref, phi_ref, phi_c0, u):
        cs = pl.ds(phi_c0, T)
        pp = phi_ref[u * 128: u * 128 + 64, cs].astype(F32).reshape(8, 8, T)
        pn = phi_ref[u * 128 + 64: u * 128 + 128, cs].astype(F32).reshape(8, 8, T)
        dpp = dphi_ref[u * 128: u * 128 + 64, :].reshape(8, 8, T)
        dpn = dphi_ref[u * 128 + 64: u * 128 + 128, :].reshape(8, 8, T)
        sp = jnp.sum(dpp * pp, axis=0)
        sn = jnp.sum(dpn * pn, axis=0)
        sp = sp + _fold(sp)
        sn = sn + _fold(sn)
        da = pp * (dpp - sp[None]) - pn * (dpn - sn[None])
        return da.reshape(64, T).astype(BF16)

    def ffn_units(r0):
        st = {}

        def ug(k):
            st[k, 'g'] = _nn(xn_v[pl.ds(r0, T), :], wg_v[:, k * FC:(k + 1) * FC])

        def uu(k):
            st[k, 'u'] = _nn(xn_v[pl.ds(r0, T), :], wu_v[:, k * FC:(k + 1) * FC])

        def ud(k):
            dh = _nt(dy_v[pl.ds(r0, T), :], wd_v[k * FC:(k + 1) * FC, :])
            gg, uv = st[k, 'g'], st[k, 'u']
            h_v[pl.ds(r0, T), k * FC:(k + 1) * FC] = (gg * uv).astype(BF16)
            dg_v[pl.ds(r0, T), k * FC:(k + 1) * FC] = (dh * uv).astype(BF16)
            du_v[pl.ds(r0, T), k * FC:(k + 1) * FC] = (dh * gg).astype(BF16)

        units = []
        for k in range(F // FC):
            units += [lambda k=k: ug(k), lambda k=k: uu(k), lambda k=k: ud(k)]
        return units

    def phase_b(t):
        c0 = pl.multiple_of(t * T, T)
        units = ffn_units(c0)

        def s1(u):
            softmax_store(pq_v, c0, phiq_v, 0, (u,))
            tmp_c[u] = _nn(kvT_b[u], phiq_v[u * 128:(u + 1) * 128, :])

        def s2(u):
            num = tmp_c[u, 0:64, :].reshape(8, 8, T)
            rden = 1.0 / (tmp_c[u, 64:72, :] + 1e-6)
            o = num * rden[None]
            dnum = doT_v[u * 64:(u + 1) * 64, pl.ds(c0, T)].reshape(8, 8, T) * rden[None]
            dd = jnp.sum(dnum * o, axis=0)
            dden = -(dd + _fold(dd))
            oT_v[u * 64:(u + 1) * 64, pl.ds(c0, T)] = o.reshape(64, T).astype(BF16)
            dnum_v[u * E: u * E + 64, :] = dnum.reshape(64, T).astype(BF16)
            dnum_v[u * E + 64: u * E + 72, :] = dden.astype(BF16)
            dn = dnum_v[u * E:(u + 1) * E, :]
            tmp_a[u * 128:(u + 1) * 128, :] = _nn(kv_b[u, :, 0:E], dn)
            dkv_acc[u, 0:E, :] += _nt(dn, phiq_v[u * 128:(u + 1) * 128, :])

        def s3(u):
            dT_v[u * 64:(u + 1) * 64, pl.ds(c0, T)] = softmax_bwd(tmp_a, phiq_v, 0, u)

        for i, un in enumerate(units):
            un()
            if i % 2 == 0 and i // 2 < U:
                s1(i // 2)
            if i % 2 == 1 and 1 <= i // 2 < U + 1:
                s2(i // 2 - 1)
            if i % 2 == 0 and 2 <= i // 2 < U + 2:
                s3(i // 2 - 2)

    _loop(NT_, phase_b)

    def meff(part):
        return _nt(xnT_v[...], dT_v[part * 512:(part + 1) * 512, :]).astype(BF16)

    def small(part, me):
        for g in range(G):
            mb = me[:, g * 128:(g + 1) * 128]
            sl = slice(part * 512 + g * 128, part * 512 + (g + 1) * 128)
            dwqkv_v[:, sl] = _nn(mb, bT_v[part * G + g]).astype(BF16)
            if part < 2:
                c_acc[part, g * 128:(g + 1) * 128, :] = _tn(wqkv_v[:, sl], mb)

    mq = meff(0)
    finish_kv(dkv_acc, dkv_b, dkvT_b)
    dxn_v[1] = jnp.zeros((T, D), F32)
    small(0, mq)

    def dx_epi(t):
        r0 = pl.multiple_of(t * T, T)
        dxn = dxn_v[t % 2]
        xn = xn_v[pl.ds(r0, T), :].astype(F32)
        m1 = jnp.mean(dxn, axis=-1, keepdims=True)
        m2 = jnp.mean(dxn * xn, axis=-1, keepdims=True)
        dx = dy_v[pl.ds(r0, T), :].astype(F32) + rstd_v[pl.ds(r0, T), :] * (dxn - m1 - xn * m2)
        dx_v[pl.ds(r0, T), :] = dx.astype(BF16)

    def phase_c(t):
        c0 = pl.multiple_of(t * T, T)
        for u in range(U):
            tmp_a[u * 128:(u + 1) * 128, :] = _nn(dkv_b[u, :, 0:E], vT_v[u * E:(u + 1) * E, pl.ds(c0, T)])
            dT_v[1024 + u * 64: 1024 + (u + 1) * 64, pl.ds(c0, T)] = _nn(
                dkvT_b[u, 0:64, :], phik_v[u * 128:(u + 1) * 128, pl.ds(c0, T)]).astype(BF16)
        for u in range(U):
            dT_v[512 + u * 64: 512 + (u + 1) * 64, pl.ds(c0, T)] = softmax_bwd(tmp_a, phik_v, c0, u)
        y = _nn(h_v[pl.ds(c0, T), :], wd_v[...]) + _tn(oT_v[:, pl.ds(c0, T)], wop_v[...])
        out_v[pl.ds(c0, T), :] = (x_v[pl.ds(c0, T), :].astype(F32) + y).astype(BF16)
        dx_epi(jnp.maximum(t - 1, 0) + (t == 0).astype(jnp.int32))
        dxn_v[t % 2] = (_tn(dT_v[:, pl.ds(c0, T)], weffT_v[...])
                        + _nt(dg_v[pl.ds(c0, T), :], wg_v[...]) + _nt(du_v[pl.ds(c0, T), :], wu_v[...]))

    _loop(NT_, phase_c)
    emit(full(out_v, out_hbm, 0))
    emit(rows(dx_v, dx_hbm, 0, S - T, 0))

    def wg_mm(f0, n=WC):
        dwg_v[:, pl.ds(f0, n)] = _nn(xnT_v[...], dg_v[:, pl.ds(f0, n)]).astype(BF16)

    def wu_mm(f0, n=WC):
        dwu_v[:, pl.ds(f0, n)] = _nn(xnT_v[...], du_v[:, pl.ds(f0, n)]).astype(BF16)

    def wd_mm(f0, n=WC):
        dwd_v[pl.ds(f0, n), :] = _tn(h_v[:, pl.ds(f0, n)], dy_v[...]).astype(BF16)

    dx_epi(NT_ - 1)
    mk = meff(1)
    dwop = _nn(oT_v[...], dy_v[...]).astype(BF16)
    small(1, mk)
    mv = meff(2)
    for g in range(G):
        dwo_v[g * 128:(g + 1) * 128, :] = _nn(p_mat, dwop[g * 128:(g + 1) * 128, :]).astype(BF16)
    rc, cc = _iota2((D, 128))
    cm = jnp.where((rc // 16) % 8 == _perm_head(cc), c_acc[0] + c_acc[1], 0.0).astype(BF16)
    re_, ce = _iota2((128, DH * DH))
    e3 = _onehot(_perm_feat(re_) == ce % 16)
    ra, ca = _iota2((D, DH * DH))
    a2 = jnp.where(ra % 16 == ca // 16, _nn(cm, e3), 0.0).astype(BF16)
    rh, ch = _iota2((D, H))
    r2t = _onehot(rh // 16 == ch)
    dwphi_v[...] = _tn(a2, r2t).astype(BF16).reshape(DH, DH, H)
    small(2, mv)
    emit(rows(dx_v, dx_hbm, S - T, T, 0))
    emit(full(dwqkv_v, dwqkv_hbm, 0))
    emit(full(dwphi_v, dwphi_hbm, 0))
    emit(full(dwo_v, dwo_hbm, 0))

    def wgrad(i):
        f0 = pl.multiple_of(i * WC, WC)
        wg_mm(f0)
        wu_mm(f0)
        wd_mm(f0)

    _loop(NWC - 1, wgrad)

    fl = (NWC - 1) * WC
    emit(cols(dwg_v, dwg_hbm, 0, fl, 0))
    emit(cols(dwu_v, dwu_hbm, 0, fl, 0))
    emit(rows(dwd_v, dwd_hbm, 0, fl, 0))
    wg_mm(fl)
    emit(cols(dwg_v, dwg_hbm, fl, WC, 0))
    wd_mm(fl)
    emit(rows(dwd_v, dwd_hbm, fl, WC, 0))
    for k in range(2):
        wu_mm(fl + k * 128, 128)
        emit(cols(dwu_v, dwu_hbm, fl + k * 128, 128, 0))

    for c in out_copies:
        c.wait()


@jax.jit
def pallas_parallel_sum__linear_kernel_hedgehog__glu_gated_bilinear__prompt_kernel(
    A_x: jax.Array,
    A_wqkv: jax.Array,
    A_w_phi: jax.Array,
    A_wo: jax.Array,
    B_x: jax.Array,
    B_w_gate: jax.Array,
    B_w_up: jax.Array,
    B_w_down: jax.Array,
    grad_out: jax.Array,
):
    del B_x
    x2 = A_x.reshape(S, D)
    dy2 = grad_out.reshape(S, D)
    wphi_t = jnp.transpose(A_w_phi, (1, 2, 0))

    vm = pltpu.VMEM
    scratch = [
        vm((S, D), BF16), vm((S, D), BF16), vm((D, 3 * D), BF16), vm((DH, DH, H), BF16), vm((D, D), BF16),
        vm((D, F), BF16), vm((D, F), BF16), vm((F, D), BF16),
        vm((S, D), BF16), vm((D, S), BF16), vm((S, 1), F32), vm((3 * D, D), BF16), vm((2 * D, D), BF16),
        vm((D, D), BF16), vm((3 * G, 128, 128), BF16),
        vm((1024, S), BF16), vm((U * E, S), BF16), vm((1024, T), BF16), vm((D, S), BF16), vm((3 * D, S), BF16),
        vm((U * E, T), BF16), vm((D, S), F32),
        vm((U, 128, 128), F32), vm((U, 128, 128), BF16), vm((U, E, 128), BF16),
        vm((U, 128, 128), F32), vm((U, 128, 128), BF16), vm((U, E, 128), BF16),
        vm((S, F), BF16), vm((S, F), BF16), vm((S, F), BF16),
        vm((1024, T), F32), vm((D, S), F32), vm((U, E, T), F32), vm((2, D, 128), F32),
        vm((2, T, D), F32),
        vm((S, D), BF16), vm((S, D), BF16), vm((D, 3 * D), BF16), vm((DH, DH, H), BF16), vm((D, D), BF16),
        vm((D, F), BF16), vm((D, F), BF16), vm((F, D), BF16),
        pltpu.SemaphoreType.DMA((5 + NT_,)),
    ]
    out_shape = (
        jax.ShapeDtypeStruct((S, D), BF16), jax.ShapeDtypeStruct((S, D), BF16),
        jax.ShapeDtypeStruct((D, 3 * D), BF16), jax.ShapeDtypeStruct((DH, DH, H), BF16),
        jax.ShapeDtypeStruct((D, D), BF16), jax.ShapeDtypeStruct((D, F), BF16),
        jax.ShapeDtypeStruct((D, F), BF16), jax.ShapeDtypeStruct((F, D), BF16),
    )
    anyspec = pl.BlockSpec(memory_space=pl.ANY)
    res = pl.pallas_call(
        _kernel,
        in_specs=[anyspec] * 8,
        out_specs=tuple([anyspec] * 8),
        out_shape=out_shape,
        scratch_shapes=scratch,
        compiler_params=pltpu.CompilerParams(vmem_limit_bytes=120 * 1024 * 1024),
    )(x2, A_wqkv, wphi_t, A_wo, B_w_gate, B_w_up, B_w_down, dy2)
    out, dx = res[0].reshape(1, S, D), res[1].reshape(1, S, D)
    dwphi = jnp.transpose(res[3], (2, 0, 1))
    return (out, dx, res[2], dwphi) + tuple(res[4:])
```
